```python
import jax
import jax.numpy as jnp

def _softmax(x, axis=-1):
    return jax.nn.softmax(x, axis=axis)
def _gelu(x):
    return jax.nn.gelu(x, approximate=True)
def _silu(x):
    return jax.nn.silu(x)
def _sigmoid(x):
    return jax.nn.sigmoid(x)
def _layernorm(x, axis=-1, eps=1e-5):
    m = jnp.mean(x, axis=axis, keepdims=True)
    v = jnp.var(x, axis=axis, keepdims=True)
    return (x - m) / jnp.sqrt(v + eps)
def _scatter_add(tgt, idx, src, axis=0):
    return tgt.at[idx].add(src)
def _segment_sum(src, seg, n):
    return jax.ops.segment_sum(src, seg, n)
class _Rng:
    def __init__(self, key):
        self._k = key
    def _next(self):
        self._k, sub = jax.random.split(self._k)
        return sub
    def normal(self, shape):
        return jax.random.normal(self._next(), shape, dtype=jnp.bfloat16)
    def randint(self, lo, hi, shape):
        return jax.random.randint(self._next(), shape, lo, hi, dtype=jnp.int32)
    def uniform(self, shape, lo=0.0, hi=1.0):
        return jax.random.uniform(self._next(), shape, jnp.bfloat16, lo, hi)
    def permutation(self, n):
        return jax.random.permutation(self._next(), n)


kernel_name = 'gated_mix__gqa_block_cached__dense_activation_relu__decode'

def _fwd_setup_inputs():
    _rng = _Rng(jax.random.key(int.from_bytes(__import__("os").urandom(4), "little")))
    _w = (lambda a: (lambda t: t.astype(jnp.bfloat16) if jnp.issubdtype(t.dtype, jnp.floating) else t)(jnp.asarray(a)))
    def _A_setup():
        B, Sq, D = 2, 1, 512
        Hq, Hkv, Sk, Dh = 32, 8, 8192, 128
        assert Hq % Hkv == 0, (Hq, Hkv)
        return {
            "x": _w((lambda *s: _rng.normal(s) * 0.05)(B, Sq, D)),
            "k_cache": _w((lambda *s: _rng.normal(s) * 0.05)(B, Hkv, Sk, Dh)),
            "v_cache": _w((lambda *s: _rng.normal(s) * 0.05)(B, Hkv, Sk, Dh)),
            "wq": _w((lambda *s: _rng.normal(s) * 0.05)(D, Hq * Dh) * (D ** -0.5)),
            "wo": _w((lambda *s: _rng.normal(s) * 0.05)(Hq * Dh, D) * ((Hq * Dh) ** -0.5)),
        }
    _A_in = _A_setup()

    def _B_setup():
        B, S, D, Dff = 2, 1, 512, 1792
        return {
            "x": _w((lambda *s: _rng.normal(s) * 0.05)(B, S, D)),
            "w1": _w((lambda *s: _rng.normal(s) * 0.05)(D, Dff)),
            "w2": _w((lambda *s: _rng.normal(s) * 0.05)(Dff, D)),
        }
    _B_in = _B_setup()

    return {
        "A_x": _A_in["x"],
        "A_k_cache": _A_in["k_cache"],
        "A_v_cache": _A_in["v_cache"],
        "A_wq": _A_in["wq"],
        "A_wo": _A_in["wo"],
        "B_x": _B_in["x"],
        "B_w1": _B_in["w1"],
        "B_w2": _B_in["w2"],
        "gate_w": _w((lambda *s: _rng.normal(s) * 0.05)(512)),
    }

def _fwd_reference(A_x, A_k_cache, A_v_cache, A_wq, A_wo, B_x, B_w1, B_w2, gate_w):
    def _A_ref(x, k_cache, v_cache, wq, wo):
        B, Sq, D = x.shape
        Hq, Dh = 32, 128
        Hkv = k_cache.shape[1]
        rep = Hq // Hkv
        q = (lambda x, *d: x.transpose(*d))((x @ wq).reshape(B, Sq, Hq, Dh), 0, 2, 1, 3)
        k = jnp.repeat(k_cache, rep, axis=1)
        v = jnp.repeat(v_cache, rep, axis=1)
        scores = jnp.einsum("bhqd,bhkd->bhqk", q, k) * (Dh ** -0.5)
        p = _softmax(scores, axis=-1)
        o = jnp.einsum("bhqk,bhkd->bhqd", p, v)
        return (lambda x, *d: x.transpose(*d))(o, 0, 2, 1, 3).reshape(B, Sq, Hq * Dh) @ wo

    def _B_ref(x, w1, w2):
        h = jnp.einsum("bsd,df->bsf", x, w1)
        zero = jnp.zeros_like(h)
        h = jnp.maximum(h, zero)
        return jnp.einsum("bsf,fd->bsd", h, w2)

    x = A_x
    g = _sigmoid((x * gate_w).sum(-1, keepdims=True))
    a = _A_ref(x, A_k_cache, A_v_cache, A_wq, A_wo)
    b = _B_ref(x, B_w1, B_w2)
    return g * a + (1 - g) * b


def setup_inputs():
    _inp = _fwd_setup_inputs()
    _gk = jax.random.fold_in(jax.random.key(int.from_bytes(__import__("os").urandom(4), "little")), 2**31 - 1)
    _shapes = [[2, 1, 512]]
    _dtypes = ['bfloat16']
    _gks = jax.random.split(_gk, len(_shapes))
    _gs = [jax.random.normal(k, s, dtype=jnp.dtype(d)) * 0.05 for k, s, d in zip(_gks, _shapes, _dtypes)]
    _inp["grad_out"] = _gs[0]
    return _inp

def reference(A_x, A_k_cache, A_v_cache, A_wq, A_wo, B_w1, B_w2, gate_w, B_x, grad_out):
    _const = dict(B_x=B_x)
    def _f(*_d):
        return _fwd_reference(**{'A_x': _d[0], 'A_k_cache': _d[1], 'A_v_cache': _d[2], 'A_wq': _d[3], 'A_wo': _d[4], 'B_w1': _d[5], 'B_w2': _d[6], 'gate_w': _d[7], **_const})
    _out, _vjp = jax.vjp(_f, A_x, A_k_cache, A_v_cache, A_wq, A_wo, B_w1, B_w2, gate_w)
    _grads = _vjp(grad_out)
    _out0 = jnp.asarray(_out)
    return (_out0, *[jnp.asarray(_g) for _g in _grads])
```

```python
import jax
import jax.numpy as jnp
from jax import lax
import jax.experimental.pallas as pl
import jax.experimental.pallas.tpu as pltpu

_B, _D = 2, 512
_HQ, _HKV, _SK, _DH = 32, 8, 8192, 128
_REP = _HQ // _HKV
_DFF = 1792
_NSTEP = _B * _HKV
_SCALE = _DH ** -0.5

_SPAN = 4096
_SPH = _SK // _SPAN
_NSTR = 8
_NGRP = _NSTEP * _SPH // _NSTR
_WROWS = 80
_NJ = -(-_SPAN // _WROWS)
_WLAST = _SPAN - (_NJ - 1) * _WROWS
_NW = 2 * _NGRP * _NJ
_Q0 = 64
_Q1 = 28
_TAIL = 448

_WQ_V = (4, _D // 32, 8, _HQ * _DH)
_WO_V = (4, _HQ * _DH // 4, _D)
_W1_V = (4, _D // 32, 8, _DFF)
_W2_V = (4, _DFF // 4, _D)

_S_X, _S_DY, _S_GW, _S_WQ, _S_WO, _S_W1, _S_W2, _S_W2T = range(8)
_S_DK, _S_DV, _S_DWQ, _S_DWO, _S_DW1, _S_DW2, _S_OUT, _S_DX, _S_DGW = range(8, 17)
_S_KV = 17
_NSEM = _S_KV + 2 * _NSTEP

_NT = (((1,), (1,)), ((), ()))
_NN = (((1,), (0,)), ((), ()))
_F32 = jnp.float32
_BF16 = jnp.bfloat16


def _dot(a, b, dims=_NN):
    return lax.dot_general(a, b, dims, preferred_element_type=_F32)


def _body(x_hbm, k_hbm, v_hbm, wq_hbm, wo_hbm, w1_hbm, w2_hbm, gw_hbm, dy_hbm,
          out_hbm, dx_hbm, dk_hbm, dv_hbm, dwq_hbm, dwo_hbm, dw1_hbm, dw2_hbm, dgw_hbm,
          x_v, dy_v, gw_v, kbuf, vbuf, wq_v, wo_v, w1_v, w2_v,
          dwq_v, dwo_v, dw1_v, dw2_v, out_v, dx_v, dgw_v,
          q_sc, do_sc, oq_sc, sem):
    copy = pltpu.make_async_copy

    cp_x = copy(x_hbm, x_v, sem.at[_S_X])
    cp_dy = copy(dy_hbm, dy_v, sem.at[_S_DY])
    cp_gw = copy(gw_hbm, gw_v, sem.at[_S_GW])
    cp_wq = copy(wq_hbm, wq_v, sem.at[_S_WQ])
    cp_wo = copy(wo_hbm, wo_v, sem.at[_S_WO])
    cp_w1 = copy(w1_hbm, w1_v, sem.at[_S_W1])
    head, tail = pl.ds(0, _DFF - _TAIL), pl.ds(_DFF - _TAIL, _TAIL)
    cp_w2 = copy(w2_hbm.at[head], w2_v.at[head], sem.at[_S_W2])
    cp_w2t = copy(w2_hbm.at[tail], w2_v.at[tail], sem.at[_S_W2T])

    def k_copy(i):
        hs = pl.ds(i * _SPH, _SPH)
        return copy(k_hbm.at[hs], kbuf.at[hs], sem.at[_S_KV + 2 * i])

    def v_copy(i):
        hs = pl.ds(i * _SPH, _SPH)
        return copy(v_hbm.at[hs], vbuf.at[hs], sem.at[_S_KV + 2 * i + 1])

    cp_wq.start()
    cp_x.start()
    cp_dy.start()
    cp_gw.start()
    cp_wo.start()
    for i in range(_NSTEP):
        k_copy(i).start()
        v_copy(i).start()
    cp_w1.start()
    cp_w2.start()
    cp_w2t.start()

    def write_kv(lo, hi):
        def issue(src, dst, slot, grp, j0, j1):
            def start(row0, rows):
                sl = (pl.ds(grp * _NSTR, _NSTR), pl.ds(row0, rows))
                copy(src.at[sl], dst.at[sl], sem.at[slot]).start()

            def one(j, c):
                start(pl.multiple_of(j * _WROWS, 16), _WROWS)
                return c
            lax.fori_loop(j0, min(j1, _NJ - 1), one, 0)
            if j1 == _NJ:
                start((_NJ - 1) * _WROWS, _WLAST)
        n = lo
        while n < hi:
            run = n // _NJ
            end = min(hi, (run + 1) * _NJ)
            src, dst, slot = (kbuf, dk_hbm, _S_DK) if run % 2 == 0 else (vbuf, dv_hbm, _S_DV)
            issue(src, dst, slot, run // 2, n - run * _NJ, end - run * _NJ)
            n = end

    def rows16(ref):
        val = ref[...].astype(_F32)
        return jnp.concatenate([jnp.broadcast_to(val[b:b + 1], (8, _D)) for b in range(_B)], axis=0)

    def small():
        xb = rows16(x_v)
        dyb = rows16(dy_v)
        gw4 = gw_v[...].astype(_F32)
        gw = jnp.concatenate([gw4[r:r + 1] for r in range(_D // 128)], axis=1)
        g = jax.nn.sigmoid(jnp.sum(xb * gw, axis=-1, keepdims=True))
        return xb, dyb, gw, g

    cp_x.wait()
    cp_dy.wait()
    cp_gw.wait()
    xb, dyb, gw, g = small()
    r4 = lax.broadcasted_iota(jnp.int32, (16, _DH), 0) % _REP

    def spread(full, dst):
        for kv in range(_HKV):
            t = [full[:, (kv * _REP + r) * _DH:(kv * _REP + r + 1) * _DH] for r in range(_REP)]
            sel = jnp.where(r4 == 0, t[0], jnp.where(r4 == 1, t[1], jnp.where(r4 == 2, t[2], t[3])))
            dst[kv] = sel[0:8]
            dst[_HKV + kv] = sel[8:16]

    cp_wq.wait()
    spread(_dot(xb.astype(_BF16), wq_v[...]), q_sc)
    cp_wo.wait()
    spread(_dot((g * dyb).astype(_BF16), wo_v[...], _NT), do_sc)

    def step(i, carry):
        k_copy(i).wait()
        v_copy(i).wait()

        @pl.when(i == _NSTEP - 1)
        def _():
            cp_w1.wait()
            cp_w2.wait()
            write_kv(0, _Q0)

        hs = pl.ds(i * _SPH, _SPH)
        q = q_sc[i]
        do = do_sc[i]
        k = kbuf[hs].reshape(_SK, _DH)
        v = vbuf[hs].reshape(_SK, _DH)
        s = _dot(q.astype(_BF16), k, _NT) * _SCALE
        dp = _dot(do.astype(_BF16), v, _NT)
        m = jnp.max(s, axis=-1, keepdims=True)
        e = jnp.exp(s - m)
        p = e * (1.0 / jnp.sum(e, axis=-1, keepdims=True))
        delta = jnp.sum(p * dp, axis=-1, keepdims=True)
        ds = p * (dp - delta) * _SCALE
        top = lax.broadcasted_iota(jnp.int32, (8, _SK), 0) < _REP
        pd = jnp.where(top, p, ds)
        pdb = pd.astype(_BF16)
        top8 = lax.broadcasted_iota(jnp.int32, (8, _DH), 0) < _REP
        oq_sc[i] = jnp.where(top8, _dot(pdb, v), _dot(pdb, k))
        wv = jnp.where(top8, do, 0.0).astype(_BF16)
        wk = jnp.where(top8, 0.0, q).astype(_BF16)
        pdt = pd.T.astype(_BF16)
        vbuf[hs] = _dot(pdt, wv).astype(_BF16).reshape(_SPH, _SPAN, _DH)
        kbuf[hs] = _dot(pdt, wk).astype(_BF16).reshape(_SPH, _SPAN, _DH)
        return carry

    lax.fori_loop(0, _NSTEP, step, 0)
    write_kv(_Q0, _Q0 + _Q1)
    cp_w2t.wait()

    xb, dyb, gw, g = small()
    rowd = lax.broadcasted_iota(jnp.int32, (16, _D), 0) % 8
    first = rowd == 0
    lo = rowd < _REP
    da = g * dyb
    db = (1.0 - g) * dyb

    h = _dot(xb.astype(_BF16), w1_v[...])
    hr = jnp.maximum(h, 0.0)
    bo = _dot(hr.astype(_BF16), w2_v[...])
    dh = _dot(db.astype(_BF16), w2_v[...], _NT)
    dh = dh * jnp.where(h > 0.0, 1.0, jnp.where(h == 0.0, 0.5, 0.0))
    dhb = dh.astype(_BF16)
    dx_ffn = _dot(dhb, w1_v[...], _NT)
    x1t = jnp.where(first, xb, 0.0).T.astype(_BF16)
    dw1_v[...] = _dot(x1t, dhb).reshape(_W1_V).astype(_BF16)
    db1 = jnp.where(first, db, 0.0).astype(_BF16)
    dw2_v[...] = _dot(hr.T.astype(_BF16), db1).astype(_BF16).reshape(_W2_V)
    write_kv(_Q0 + _Q1, _Q0 + 2 * _Q1)

    r4 = lax.broadcasted_iota(jnp.int32, (16, _DH), 0) % _REP
    tiles = []
    for kv in range(_HKV):
        t = jnp.concatenate([oq_sc[kv], oq_sc[_HKV + kv]], axis=0)
        for r in range(_REP):
            tiles.append(jnp.where(r4 == r, t, 0.0))
    w = jnp.concatenate(tiles, axis=1)
    wb = w.astype(_BF16)
    a_rows = jnp.where(lo, _dot(wb, wo_v[...]), 0.0)
    dx_rows = jnp.where(lo, 0.0, _dot(wb, wq_v[...], _NT))
    write_kv(_Q0 + 2 * _Q1, _Q0 + 3 * _Q1)
    xmt = jnp.where(lo, 0.0, xb).T.astype(_BF16)
    dwq_v[...] = _dot(xmt, wb).reshape(_WQ_V).astype(_BF16)
    write_kv(_Q0 + 3 * _Q1, _Q0 + 4 * _Q1)
    dam = jnp.where(lo, da, 0.0).astype(_BF16)
    dwo_v[...] = _dot(w.T.astype(_BF16), dam).astype(_BF16).reshape(_WO_V)

    dgw = jnp.zeros((1, _D), _F32)
    outs, dxs = [], []
    for b in range(_B):
        a_b = jnp.sum(a_rows[8 * b:8 * b + 8], axis=0, keepdims=True)
        dxa_b = jnp.sum(dx_rows[8 * b:8 * b + 8], axis=0, keepdims=True)
        g_b = g[8 * b:8 * b + 1]
        bo_b = bo[8 * b:8 * b + 1]
        outs.append(g_b * a_b + (1.0 - g_b) * bo_b)
        dsg = jnp.sum(dyb[8 * b:8 * b + 1] * (a_b - bo_b), axis=-1, keepdims=True) * g_b * (1.0 - g_b)
        dxs.append(dxa_b + dx_ffn[8 * b:8 * b + 1] + dsg * gw)
        dgw = dgw + dsg * xb[8 * b:8 * b + 1]
    out_v[...] = jnp.concatenate(outs, axis=0).astype(_BF16)
    dx_v[...] = jnp.concatenate(dxs, axis=0).astype(_BF16)
    dgw_v[...] = jnp.concatenate(
        [dgw[:, r * 128:(r + 1) * 128] for r in range(_D // 128)], axis=0).astype(_BF16)

    cp_out = copy(out_v, out_hbm, sem.at[_S_OUT])
    cp_dx = copy(dx_v, dx_hbm, sem.at[_S_DX])
    cp_dgw = copy(dgw_v, dgw_hbm, sem.at[_S_DGW])
    cp_out.start()
    cp_dx.start()
    cp_dgw.start()
    write_kv(_Q0 + 4 * _Q1, _NW)

    def start_w(src, dst, slot, r0, rows, c0, cols):
        sl = (slice(None), pl.ds(r0, rows), pl.ds(c0, cols))
        copy(src.at[sl], dst.at[sl], sem.at[slot]).start()

    def start_g(src, dst, slot, r, c0, cols):
        sl = (slice(None), r, slice(None), pl.ds(c0, cols))
        copy(src.at[sl], dst.at[sl], sem.at[slot]).start()

    def qo_body(r, c):
        for cc in range(4):
            start_g(dwq_v, dwq_hbm, _S_DWQ, r, cc * 1024, 1024)
            start_w(dwo_v, dwo_hbm, _S_DWO, pl.multiple_of((r * 4 + cc) * 16, 16), 16, 0, _D)
        return c

    lax.fori_loop(0, _WQ_V[1], qo_body, 0)

    def ff_body(r, c):
        for cc in range(2):
            start_g(dw1_v, dw1_hbm, _S_DW1, r, cc * 896, 896)
            start_w(dw2_v, dw2_hbm, _S_DW2, pl.multiple_of((r * 2 + cc) * 16, 16), 16, 0, _D)
        return c

    lax.fori_loop(0, _W2_V[1] // 32, ff_body, 0)
    for r in range(_W2_V[1] // 32, _W1_V[1]):
        for cc in range(2):
            start_g(dw1_v, dw1_hbm, _S_DW1, r, cc * 896, 896)

    cp_out.wait()
    cp_dx.wait()
    cp_dgw.wait()
    copy(kbuf, dk_hbm, sem.at[_S_DK]).wait()
    copy(vbuf, dv_hbm, sem.at[_S_DV]).wait()
    copy(dwq_v, dwq_hbm, sem.at[_S_DWQ]).wait()
    copy(dwo_v, dwo_hbm, sem.at[_S_DWO]).wait()
    copy(dw2_v, dw2_hbm, sem.at[_S_DW2]).wait()
    copy(dw1_v, dw1_hbm, sem.at[_S_DW1]).wait()


def _kernel(*refs):
    pl.run_scoped(lambda sem: _body(*refs, sem), pltpu.SemaphoreType.DMA((_NSEM,)))


@jax.jit
def pallas_gated_mix__gqa_block_cached__dense_activation_relu__decode_kernel(
    A_x: jax.Array,
    A_k_cache: jax.Array,
    A_v_cache: jax.Array,
    A_wq: jax.Array,
    A_wo: jax.Array,
    B_x: jax.Array,
    B_w1: jax.Array,
    B_w2: jax.Array,
    gate_w: jax.Array,
    grad_out: jax.Array,
):
    del B_x
    kv_shape = (_NSTEP * _SPH, _SPAN, _DH)
    gw_shape = (_D // 128, 128)
    any_spec = pl.BlockSpec(memory_space=pl.ANY)
    sds = jax.ShapeDtypeStruct
    out_shape = (
        sds((_B, _D), _BF16), sds((_B, _D), _BF16),
        sds(kv_shape, _BF16), sds(kv_shape, _BF16),
        sds(_WQ_V, _BF16), sds(_WO_V, _BF16), sds(_W1_V, _BF16), sds(_W2_V, _BF16),
        sds(gw_shape, _BF16),
    )
    vm = pltpu.VMEM
    scratch = [
        vm((_B, _D), _BF16), vm((_B, _D), _BF16), vm(gw_shape, _BF16),
        vm(kv_shape, _BF16), vm(kv_shape, _BF16),
        vm(A_wq.shape, _BF16), vm(A_wo.shape, _BF16), vm(B_w1.shape, _BF16), vm(B_w2.shape, _BF16),
        vm(_WQ_V, _BF16), vm(_WO_V, _BF16), vm(_W1_V, _BF16), vm(_W2_V, _BF16),
        vm((_B, _D), _BF16), vm((_B, _D), _BF16), vm(gw_shape, _BF16),
        vm((_NSTEP, 8, _DH), _F32), vm((_NSTEP, 8, _DH), _F32), vm((_NSTEP, 8, _DH), _F32),
    ]
    out, dx, dk, dv, dwq, dwo, dw1, dw2, dgw = pl.pallas_call(
        _kernel,
        in_specs=[any_spec] * 9,
        out_specs=[any_spec] * 9,
        out_shape=out_shape,
        scratch_shapes=scratch,
        compiler_params=pltpu.CompilerParams(vmem_limit_bytes=110 * 1024 * 1024),
    )(A_x.reshape(_B, _D), A_k_cache.reshape(kv_shape), A_v_cache.reshape(kv_shape),
      A_wq, A_wo, B_w1, B_w2, gate_w.reshape(gw_shape), grad_out.reshape(_B, _D))
    return (out.reshape(A_x.shape), dx.reshape(A_x.shape),
            dk.reshape(A_k_cache.shape), dv.reshape(A_v_cache.shape),
            dwq.reshape(A_wq.shape), dwo.reshape(A_wo.shape),
            dw1.reshape(B_w1.shape), dw2.reshape(B_w2.shape), dgw.reshape(gate_w.shape))
```
